```python
import os as _os
_os.environ.setdefault("JAX_PLATFORMS", "cpu")
import jax
import jax.numpy as jnp

def _softmax(x, axis=-1):
    return jax.nn.softmax(x, axis=axis)
def _gelu(x):
    return jax.nn.gelu(x, approximate=True)
def _silu(x):
    return jax.nn.silu(x)
def _sigmoid(x):
    return jax.nn.sigmoid(x)
def _layernorm(x, axis=-1, eps=1e-5):
    m = jnp.mean(x, axis=axis, keepdims=True)
    v = jnp.var(x, axis=axis, keepdims=True)
    return (x - m) / jnp.sqrt(v + eps)
def _scatter_add(tgt, idx, src, axis=0):
    return tgt.at[idx].add(src)
def _segment_sum(src, seg, n):
    return jax.ops.segment_sum(src, seg, n)
class _Rng:
    def __init__(self, key):
        self._k = key
    def _next(self):
        self._k, sub = jax.random.split(self._k)
        return sub
    def normal(self, shape):
        return jax.random.normal(self._next(), shape, dtype=jnp.bfloat16)
    def randint(self, lo, hi, shape):
        return jax.random.randint(self._next(), shape, lo, hi, dtype=jnp.int32)
    def uniform(self, shape, lo=0.0, hi=1.0):
        return jax.random.uniform(self._next(), shape, jnp.bfloat16, lo, hi)
    def permutation(self, n):
        return jax.random.permutation(self._next(), n)


kernel_name = 'concat_heads__ssm_conv_s4__linear_attn_block__prompt'

def setup_inputs():
    _rng = _Rng(jax.random.key(int.from_bytes(__import__("os").urandom(4), "little")))
    _w = (lambda a: (lambda t: t.astype(jnp.bfloat16) if jnp.issubdtype(t.dtype, jnp.floating) else t)(jnp.asarray(a)))
    def _A_setup():
        B, L, D, N = 1, 2048, 512, 128
        A_re = -jnp.exp((lambda *s: _rng.normal(s) * 0.1)(D, N))
        A_im = jnp.pi * (lambda *s: _rng.normal(s) * 0.1)(D, N)
        B_re = (lambda *s: _rng.normal(s) * 0.1)(D, N)
        B_im = (lambda *s: _rng.normal(s) * 0.1)(D, N)
        C_re = (lambda *s: _rng.normal(s) * 0.1)(D, N)
        C_im = (lambda *s: _rng.normal(s) * 0.1)(D, N)
        log_dt = (lambda *s: _rng.normal(s) * 0.1)(D) * 0.5 - 4.0
        Dskip = (lambda *s: _rng.normal(s) * 0.05)(D)
        return {
            "u": _w((lambda *s: _rng.normal(s) * 0.05)(B, L, D)),
            "A_re": _w(A_re),
            "A_im": _w(A_im),
            "B_re": _w(B_re),
            "B_im": _w(B_im),
            "C_re": _w(C_re),
            "C_im": _w(C_im),
            "log_dt": _w(log_dt),
            "Dskip": _w(Dskip),
        }
    _A_in = _A_setup()

    def _B_setup():
        B, S, D = 1, 2048, 512
        return {
            "x": _w((lambda *s: _rng.normal(s) * 0.05)(B, S, D)),
            "wqkv": _w((lambda *s: _rng.normal(s) * 0.4)(D, 3 * D)),
            "wo": _w((lambda *s: _rng.normal(s) * 0.05)(D, D)),
        }
    _B_in = _B_setup()

    return {
        "A_u": _A_in["u"],
        "A_A_re": _A_in["A_re"],
        "A_A_im": _A_in["A_im"],
        "A_B_re": _A_in["B_re"],
        "A_B_im": _A_in["B_im"],
        "A_C_re": _A_in["C_re"],
        "A_C_im": _A_in["C_im"],
        "A_log_dt": _A_in["log_dt"],
        "A_Dskip": _A_in["Dskip"],
        "B_x": _B_in["x"],
        "B_wqkv": _B_in["wqkv"],
        "B_wo": _B_in["wo"],
    }

def reference(A_u, A_A_re, A_A_im, A_B_re, A_B_im, A_C_re, A_C_im, A_log_dt, A_Dskip, B_x, B_wqkv, B_wo):
    def _A_ref(u, A_re, A_im, B_re, B_im, C_re, C_im, log_dt, Dskip):
        Bsz, L, D = u.shape
        dt = jnp.exp(log_dt)[:, None]
        A = A_re + 1j * A_im
        Bc = B_re + 1j * B_im
        Cc = C_re + 1j * C_im
        logdA = dt * A
        dB = dt * Bc
        l = (lambda x, dt: x.astype(dt))(jnp.arange(L), A_re.dtype)
        P = jnp.exp(logdA[:, :, None] * l[None, None, :])
        K = jnp.einsum("dn,dnl,dn->dl", Cc, P, dB).real
        L2 = 2 * L
        Kp = jnp.pad(K, ((0, 0), (0, L)))
        up = (lambda x, *d: x.transpose(*d))(u, 0, 2, 1)
        up = jnp.pad(up, ((0, 0), (0, 0), (0, L)))
        Kf = (lambda x, axes=(-2,-1): jnp.fft.rfft2(x.astype(jnp.float32), axes=axes))(Kp[:, None, :], axes=(-2, -1))
        Uf = (lambda x, axes=(-2,-1): jnp.fft.rfft2(x.astype(jnp.float32), axes=axes))(up[:, :, None, :], axes=(-2, -1))
        Yf = Uf * Kf[None, :, :, :]
        y = (lambda x, s, axes=(-2,-1): jnp.fft.irfft2(x, s=s, axes=axes).astype(jnp.bfloat16))(Yf, (1, L2), axes=(-2, -1))[:, :, 0, :L]
        y = (lambda x, *d: x.transpose(*d))(y, 0, 2, 1) + u * Dskip[None, None, :]
        return y

    def _B_ref(x, wqkv, wo):
        B, S, D = x.shape
        H = 32; Dh = D // H
        qkv = (lambda x, *d: x.transpose(*d))((x @ wqkv).reshape(B, S, 3, H, Dh), 2, 0, 3, 1, 4)
        q, k, v = qkv[0], qkv[1], qkv[2]
        phi = lambda t: jnp.where(t > 0, t + 1, jnp.exp(t)) + 1e-6
        pq, pk = phi(q), phi(k)
        kv = jnp.einsum("bhsd,bhse->bhde", pk, v)
        z = jnp.einsum("bhsd->bhd", pk)
        num = jnp.einsum("bhqd,bhde->bhqe", pq, kv)
        den = jnp.einsum("bhqd,bhd->bhq", pq, z)[..., None] + 1e-6
        o = num / den
        return (lambda x, *d: x.transpose(*d))(o, 0, 2, 1, 3).reshape(B, S, D) @ wo

    a = _A_ref(A_u, A_A_re, A_A_im, A_B_re, A_B_im, A_C_re, A_C_im, A_log_dt, A_Dskip)
    b = _B_ref(B_x, B_wqkv, B_wo)
    return jnp.concatenate([a, b], axis=-1)
```

```python
import numpy as np
import ml_dtypes
import jax
import jax.numpy as jnp
from jax import lax
import jax.experimental.pallas as pl
import jax.experimental.pallas.tpu as pltpu

L, D, N, T = 2048, 512, 128, 128
BF, F32 = jnp.bfloat16, jnp.float32


def _tables():
    n0 = np.arange(64)[:, None, None]
    k1 = np.arange(64)[None, :, None]
    n1 = np.arange(32)[None, None, :]
    e = np.exp(-2j * np.pi * (n1 * k1 / 64 + n0 * k1 / 4096))
    f1 = np.concatenate([e.real, e.imag], 1)
    g = np.exp(-2j * np.pi * np.outer(np.arange(64), np.arange(64)) / 64)
    g2 = np.block([[g.real, -g.imag], [g.imag, g.real]])
    i2 = np.block([[g.real, g.imag], [-g.imag, g.real]])
    i1 = np.transpose(f1, (0, 2, 1)) / 4096
    c = lambda a: a.astype(np.float32).astype(ml_dtypes.bfloat16)
    return c(f1), c(g2), c(i2), c(i1)


_F1, _G2, _I2, _I1 = _tables()
_SEGS = ((0, 1, 256), (256, 2, 128), (512, 4, 128), (1024, 8, 129))
_LQ = np.arange(L).astype(np.float32).astype(ml_dtypes.bfloat16).astype(np.int64)


def _dot(a, b):
    return jnp.dot(a, b, preferred_element_type=F32)


def _kern(u_ref, are, aim, bre, bim, cre, cim, ldt, dsk, x_ref, wq, wk, wv, wo,
          f1, g2, i2, i1, o_ref, kd, kf, uf, z, kh, ob):
    j = pl.program_id(0)
    dt = jnp.exp(ldt[...].astype(F32)).astype(BF).astype(F32)
    ar = dt * are[...].astype(F32)
    ai = dt * aim[...].astype(F32)
    br = dt * bre[...].astype(F32)
    bi = dt * bim[...].astype(F32)
    cr, ci = cre[...].astype(F32), cim[...].astype(F32)
    wr, wi = cr * br - ci * bi, cr * bi + ci * br

    def val(l, m, c, s):
        return m * (wr * c - wi * s)

    e = jnp.exp(ar)
    lr, li = e * jnp.cos(ai), e * jnp.sin(ai)
    e = jnp.exp(ar * 256.0)
    hr, hi = e * jnp.cos(ai * 256.0), e * jnp.sin(ai * 256.0)
    sr, si = wr, wi
    off = 0
    for l0, st, cnt in _SEGS:
        p, q = 2 * lr, lr * lr + li * li
        xa, xb = sr, sr * lr - si * li
        ng = (cnt + 7) // 8
        for h in range(2):
            sl = slice(64 * h, 64 * h + 64)

            def grp(gi, c, p=p[sl], q=q[sl], h=h, off=off):
                x0, x1 = c
                out = jnp.zeros((8, T), F32)
                sub = lax.broadcasted_iota(jnp.int32, (8, T), 0)
                for r in range(8):
                    row = x0.reshape(8, 8, T).sum(0).sum(0, keepdims=True)
                    out = jnp.where(sub == r, row, out)
                    x0, x1 = x1, p * x1 - q * x0
                ds = pl.ds(pl.multiple_of(off + gi * 8, 8), 8)
                kd[ds, :] = out if h == 0 else kd[ds, :] + out
                return x0, x1

            lax.fori_loop(0, ng, grp, (xa[sl], xb[sl]))
        off += cnt
        sr, si = sr * hr - si * hi, sr * hi + si * hr
        lr, li = lr * lr - li * li, 2 * lr * li
        if l0:
            hr, hi = hr * hr - hi * hi, 2 * hr * hi
    kf[0:256, :] = kd[0:256, :]
    off = 256
    for l0, st, cnt in _SEGS[1:]:
        for r in range(2 * st):
            s = int(_LQ[l0 + r] - l0) // st
            kf[pl.ds(l0 + r, 64, stride=2 * st), :] = kd[pl.ds(off + s, 64, stride=2), :]
        off += 128
    u = u_ref[...]
    uf[...] = u.astype(F32)

    def stage1(src):
        def b(n0, _):
            r = _dot(f1[n0], src[pl.ds(n0, 32, stride=64), :].astype(BF))
            z[pl.ds(n0, 64, stride=136), :] = r[:64]
            z[pl.ds(n0 + 64, 64, stride=136), :] = r[64:]
            return 0
        lax.fori_loop(0, 64, b, 0, unroll=16)

    def rows(k1):
        return pl.ds(pl.multiple_of(k1 * 136, 8), 128)

    stage1(kf)

    def s2k(k1, _):
        kh[rows(k1), :] = _dot(g2[...], z[rows(k1), :].astype(BF))
        return 0
    lax.fori_loop(0, 64, s2k, 0, unroll=16)
    stage1(uf)

    def s2u(k1, _):
        a = _dot(g2[...], z[rows(k1), :].astype(BF))
        k = kh[rows(k1), :]
        y = jnp.concatenate([a[:64] * k[:64] - a[64:] * k[64:],
                             a[:64] * k[64:] + a[64:] * k[:64]], 0)
        z[rows(k1), :] = _dot(i2[...], y.astype(BF))
        return 0
    lax.fori_loop(0, 64, s2u, 0, unroll=16)

    def fin(n0, _):
        h = jnp.concatenate([z[pl.ds(n0, 64, stride=136), :],
                             z[pl.ds(n0 + 64, 64, stride=136), :]], 0)
        kf[pl.ds(n0, 32, stride=64), :] = _dot(i1[n0], h.astype(BF))
        return 0
    lax.fori_loop(0, 64, fin, 0, unroll=16)
    col = pl.ds(pl.multiple_of(j * T, T), T)
    ud = (u.astype(F32) * dsk[...].astype(F32)).astype(BF).astype(F32)
    o_ref[:, col] = (kf[...].astype(BF).astype(F32) + ud).astype(BF)

    x = x_ref[...]

    def phi(t):
        t = t.astype(BF).astype(F32)
        return (jnp.where(t > 0, t + 1, jnp.exp(t)) + 1e-6).astype(BF)

    pq, pk = phi(_dot(x, wq[...])), phi(_dot(x, wk[...]))
    v = _dot(x, wv[...]).astype(BF)
    tn = (((0,), (0,)), ((), ()))
    kv = lax.dot_general(pk, v, tn, preferred_element_type=F32)
    zz = lax.dot_general(pk, jnp.ones((L, T), BF), tn, preferred_element_type=F32)
    same = (lax.broadcasted_iota(jnp.int32, (T, T), 0) // 16
            == lax.broadcasted_iota(jnp.int32, (T, T), 1) // 16)
    num = _dot(pq, jnp.where(same, kv, 0).astype(BF))
    den = _dot(pq, jnp.where(same, zz, 0).astype(BF)) + 1e-6
    ob[:, col] = (num / den).astype(BF)

    @pl.when(j == D // T - 1)
    def _():
        o_ref[:, D:] = _dot(ob[...], wo[...]).astype(BF)


@jax.jit
def pallas_concat_heads__ssm_conv_s4__linear_attn_block__prompt_kernel(
        A_u, A_A_re, A_A_im, A_B_re, A_B_im, A_C_re, A_C_im, A_log_dt, A_Dskip,
        B_x, B_wqkv, B_wo):
    nt = D // T
    colb = lambda r: pl.BlockSpec((r, T), lambda j: (0, j))
    full = lambda a: pl.BlockSpec(a.shape, lambda j: (0,) * a.ndim)
    w = lambda o: pl.BlockSpec((D, T), lambda j: (0, j + o * nt))
    x = B_x.reshape(L, D)
    ps = [a.T for a in (A_A_re, A_A_im, A_B_re, A_B_im, A_C_re, A_C_im)]
    out = pl.pallas_call(
        _kern,
        grid=(nt,),
        in_specs=[colb(L)] + [colb(N)] * 6 + [colb(1)] * 2
        + [full(x), w(0), w(1), w(2), full(B_wo)]
        + [full(t) for t in (_F1, _G2, _I2, _I1)],
        out_specs=pl.BlockSpec((L, 2 * D), lambda j: (0, 0)),
        out_shape=jax.ShapeDtypeStruct((L, 2 * D), BF),
        scratch_shapes=[pltpu.VMEM((648, T), F32), pltpu.VMEM((L, T), F32),
                        pltpu.VMEM((L, T), F32), pltpu.VMEM((8704, T), F32),
                        pltpu.VMEM((8704, T), F32), pltpu.VMEM((L, D), BF)],
        compiler_params=pltpu.CompilerParams(
            dimension_semantics=("arbitrary",), vmem_limit_bytes=100 << 20),
    )(A_u.reshape(L, D), *ps, A_log_dt.reshape(1, D), A_Dskip.reshape(1, D),
      x, B_wqkv, B_wqkv, B_wqkv, B_wo, _F1, _G2, _I2, _I1)
    return out.reshape(1, L, 2 * D)
```
